```python
import os as _os
_os.environ.setdefault("JAX_PLATFORMS", "cpu")
import jax
import jax.numpy as jnp

def _softmax(x, axis=-1):
    return jax.nn.softmax(x, axis=axis)
def _gelu(x):
    return jax.nn.gelu(x, approximate=True)
def _silu(x):
    return jax.nn.silu(x)
def _sigmoid(x):
    return jax.nn.sigmoid(x)
def _layernorm(x, axis=-1, eps=1e-5):
    m = jnp.mean(x, axis=axis, keepdims=True)
    v = jnp.var(x, axis=axis, keepdims=True)
    return (x - m) / jnp.sqrt(v + eps)
def _scatter_add(tgt, idx, src, axis=0):
    return tgt.at[idx].add(src)
def _segment_sum(src, seg, n):
    return jax.ops.segment_sum(src, seg, n)
class _Rng:
    def __init__(self, key):
        self._k = key
    def _next(self):
        self._k, sub = jax.random.split(self._k)
        return sub
    def normal(self, shape):
        return jax.random.normal(self._next(), shape, dtype=jnp.bfloat16)
    def randint(self, lo, hi, shape):
        return jax.random.randint(self._next(), shape, lo, hi, dtype=jnp.int32)
    def uniform(self, shape, lo=0.0, hi=1.0):
        return jax.random.uniform(self._next(), shape, jnp.bfloat16, lo, hi)
    def permutation(self, n):
        return jax.random.permutation(self._next(), n)


kernel_name = 'parallel_sum__grouped_kv_mqa__dense_activation_silu__prompt'

def setup_inputs():
    _rng = _Rng(jax.random.key(int.from_bytes(__import__("os").urandom(4), "little")))
    _w = (lambda a: (lambda t: t.astype(jnp.bfloat16) if jnp.issubdtype(t.dtype, jnp.floating) else t)(jnp.asarray(a)))
    def _A_setup():
        B, S, D, H = 1, 2048, 512, 32
        Dh = D // H
        return {
            "x": _w((lambda *s: _rng.normal(s) * 0.05)(B, S, D)),
            "wq": _w((lambda *s: _rng.normal(s) * 0.05)(D, H * Dh)),
            "wk": _w((lambda *s: _rng.normal(s) * 0.05)(D, Dh)),
            "wv": _w((lambda *s: _rng.normal(s) * 0.05)(D, Dh)),
            "wo": _w((lambda *s: _rng.normal(s) * 0.05)(H * Dh, D)),
        }
    _A_in = _A_setup()

    def _B_setup():
        B, S, D, F = 1, 2048, 512, 1376
        return {
            "x": _w((lambda *s: _rng.normal(s) * 0.05)(B, S, D)),
            "w1": _w((lambda *s: _rng.normal(s) * 0.05)(D, F) * (D ** -0.5)),
            "w2": _w((lambda *s: _rng.normal(s) * 0.05)(F, D) * (F ** -0.5)),
        }
    _B_in = _B_setup()

    return {
        "A_x": _A_in["x"],
        "A_wq": _A_in["wq"],
        "A_wk": _A_in["wk"],
        "A_wv": _A_in["wv"],
        "A_wo": _A_in["wo"],
        "B_x": _B_in["x"],
        "B_w1": _B_in["w1"],
        "B_w2": _B_in["w2"],
    }

def reference(A_x, A_wq, A_wk, A_wv, A_wo, B_x, B_w1, B_w2):
    def _A_ref(x, wq, wk, wv, wo):
        B, S, D = x.shape
        H = 32
        Dh = D // H
        q = (lambda x, *d: x.transpose(*d))((x @ wq).reshape(B, S, H, Dh), 0, 2, 1, 3)
        k = x @ wk
        v = x @ wv
        scores = jnp.einsum("bhqd,bkd->bhqk", q, k) * (Dh ** -0.5)
        p = _softmax(scores, axis=-1)
        o = jnp.einsum("bhqk,bkd->bhqd", p, v)
        return (lambda x, *d: x.transpose(*d))(o, 0, 2, 1, 3).reshape(B, S, H * Dh) @ wo

    def _B_ref(x, w1, w2):
        h = jnp.einsum("bsd,df->bsf", x, w1)
        h = _silu(h)
        out = jnp.einsum("bsf,fd->bsd", h, w2)
        return out

    x = A_x
    xn = _layernorm(x, axis=-1)
    return x + _A_ref(xn, A_wq, A_wk, A_wv, A_wo) + _B_ref(xn, B_w1, B_w2)
```

```python
import jax
import jax.numpy as jnp
from jax import lax
import jax.experimental.pallas as pl
import jax.experimental.pallas.tpu as pltpu

S, D, H, DH, F = 2048, 512, 32, 16, 1376
LOG2E = 1.4426950408889634
NT = (((1,), (1,)), ((), ()))

def _ln(x):
    x = x.astype(jnp.float32)
    m = jnp.mean(x, axis=-1, keepdims=True)
    xc = x - m
    v = jnp.mean(xc * xc, axis=-1, keepdims=True)
    return (xc * lax.rsqrt(v + 1e-5))

def make(TQ=512, CH=128, VM=16, NIT=15, ORD=0, NS=1, FL={}, RC=256, KD=16, C1=1):
    NC = S // CH
    def kernel(x_ref, wq_ref, wkt_ref, wvt_ref, wo_h, w1t_h, w2_h, o_ref,
               k_scr, vt_scr, qt_scr, ot_scr, sa, sb, wo_ref, w1t_ref, w2_ref, sems):
        i = pl.program_id(0)

        cps = [pltpu.make_async_copy(a, b, sems.at[n]) for n, (a, b) in enumerate(((wo_h, wo_ref), (w1t_h, w1t_ref), (w2_h, w2_ref)))]

        @pl.when(i == 0)
        def _():
            for cp in cps:
                cp.start()
            if KD > DH: qt_scr[...] = jnp.zeros(qt_scr.shape, qt_scr.dtype)
            wk = jnp.concatenate([wkt_ref[...], jnp.zeros((128 - DH, D), jnp.bfloat16)], axis=0)
            wv = jnp.concatenate([wvt_ref[...], jnp.zeros((DH, D), jnp.bfloat16)], axis=0) if VM > DH else wvt_ref[...]
            def body(c, carry):
                r = pl.multiple_of(c * CH, CH)
                xn = _ln(x_ref[pl.ds(r, CH), :]).astype(jnp.bfloat16)
                k = lax.dot_general(xn, wk, NT, preferred_element_type=jnp.float32)
                k_scr[pl.ds(r, CH), :] = k[:, :KD].astype(jnp.bfloat16)
                vt = lax.dot_general(wv, xn, NT, preferred_element_type=jnp.float32)
                row = lax.broadcasted_iota(jnp.int32, vt.shape, 0)
                vt_scr[c] = jnp.where(row == DH, 1.0, vt).astype(jnp.bfloat16)
                return carry
            lax.fori_loop(0, NC, body, 0)

        r0 = pl.multiple_of(i * TQ, TQ)
        xb = x_ref[pl.ds(r0, TQ), :]
        xn = _ln(xb).astype(jnp.bfloat16)
        q = jnp.dot(xn, wq_ref[...], preferred_element_type=jnp.float32) * (0.25 * LOG2E)
        qt_scr[:, :DH, :] = q.T.astype(jnp.bfloat16).reshape(H, DH, TQ)

        def step(h1, s1, h2, s2, m2):
            m1 = None
            acc = None
            if h1 is not None:
                qt = qt_scr[h1]
            for c in range(NC):
                sl = slice(c * CH, (c + 1) * CH)
                if ORD == 0:
                    if h1 is not None and c % C1 == 0:
                        sl1 = slice(c * CH, (c + C1) * CH)
                        st = jnp.dot(k_scr[sl1, :], qt, preferred_element_type=jnp.float32)
                        s1[sl1, :] = st
                        mc = jnp.max(st.reshape(C1 * CH // 8, 8, TQ), axis=0)
                        m1 = mc if m1 is None else jnp.maximum(m1, mc)
                if h2 is not None:
                    pf = jnp.exp2(s2[sl, :] - m2)
                    p = pf.astype(jnp.bfloat16)
                    if VM == DH:
                        lc = jnp.sum(pf.reshape(CH // 8, 8, TQ), axis=0)
                        l = lc if acc is None else l + lc
                    t = jnp.dot(vt_scr[c], p, preferred_element_type=jnp.float32)
                    acc = t if acc is None else acc + t
                if ORD == 1:
                    if h1 is not None and c % C1 == 0:
                        sl1 = slice(c * CH, (c + C1) * CH)
                        st = jnp.dot(k_scr[sl1, :], qt, preferred_element_type=jnp.float32)
                        s1[sl1, :] = st
                        mc = jnp.max(st.reshape(C1 * CH // 8, 8, TQ), axis=0)
                        m1 = mc if m1 is None else jnp.maximum(m1, mc)
            if h2 is not None:
                hr = pl.multiple_of(h2 * DH, DH)
                ot_scr[pl.ds(hr, DH), :] = acc[:DH] / (acc[DH:DH + 1] if VM > DH else jnp.sum(l, axis=0, keepdims=True))
            if h1 is not None:
                return jnp.max(m1, axis=0, keepdims=True)

        m = step(0, sa, None, None, None)
        def body(j, m):
            m = step(2 * j + 1, sb, 2 * j, sa, m)
            m = step(2 * j + 2, sa, 2 * j + 1, sb, m)
            return m
        m = lax.fori_loop(0, NIT, body, m)
        m = step(H - 1, sb, H - 2, sa, m)
        step(None, None, H - 1, sb, m)

        @pl.when(i == 0)
        def _():
            for cp in cps:
                cp.wait()

        o = ot_scr[...].T.astype(jnp.bfloat16)
        for r in range(TQ // RC):
            rs = slice(r * RC, (r + 1) * RC)
            att = jnp.dot(o[rs], wo_ref[...], preferred_element_type=jnp.float32)
            hh = lax.dot_general(xn[rs], w1t_ref[...], NT, preferred_element_type=jnp.float32)
            hh = hh * (0.5 * jnp.tanh(0.5 * hh) + 0.5)
            ff = jnp.dot(hh.astype(jnp.bfloat16), w2_ref[...], preferred_element_type=jnp.float32)
            o_ref[rs, :] = (xb[rs].astype(jnp.float32) + att + ff).astype(o_ref.dtype)

    @jax.jit
    def f(A_x, A_wq, A_wk, A_wv, A_wo, B_x, B_w1, B_w2):
        x = A_x.reshape(S, D)
        full = lambda shp: pl.BlockSpec(shp, lambda i: (0,) * len(shp))
        ANY = pl.BlockSpec(memory_space=pl.ANY)
        out = pl.pallas_call(
            kernel,
            grid=(S // TQ,),
            in_specs=[full((S, D)), full((D, D)), full((DH, D)), full((DH, D)), ANY, ANY, ANY],
            out_specs=pl.BlockSpec((TQ, D), lambda i: (i, 0)),
            out_shape=jax.ShapeDtypeStruct((S, D), A_x.dtype),
            scratch_shapes=[
                pltpu.VMEM((S, KD), jnp.bfloat16),
                pltpu.VMEM((NC, VM, CH), jnp.bfloat16),
                pltpu.VMEM((H, KD, TQ), jnp.bfloat16),
                pltpu.VMEM((D, TQ), jnp.float32),
                pltpu.VMEM((S, TQ), jnp.float32),
                pltpu.VMEM((S, TQ), jnp.float32),
                pltpu.VMEM((D, D), jnp.bfloat16),
                pltpu.VMEM((F, D), jnp.bfloat16),
                pltpu.VMEM((F, D), jnp.bfloat16),
                pltpu.SemaphoreType.DMA((3,)),
            ],
            compiler_params=pltpu.CompilerParams(dimension_semantics=("arbitrary",), flags=FL, vmem_limit_bytes=100 * 1024 * 1024),
        )(x, A_wq, A_wk.T, A_wv.T, A_wo, B_w1.T, B_w2)
        return out.reshape(1, S, D)
    return f

pallas_parallel_sum__grouped_kv_mqa__dense_activation_silu__prompt_kernel = make()
```
